```python
import jax
import jax.numpy as jnp

def _softmax(x, axis=-1):
    return jax.nn.softmax(x, axis=axis)
def _gelu(x):
    return jax.nn.gelu(x, approximate=True)
def _silu(x):
    return jax.nn.silu(x)
def _sigmoid(x):
    return jax.nn.sigmoid(x)
def _layernorm(x, axis=-1, eps=1e-5):
    m = jnp.mean(x, axis=axis, keepdims=True)
    v = jnp.var(x, axis=axis, keepdims=True)
    return (x - m) / jnp.sqrt(v + eps)
def _scatter_add(tgt, idx, src, axis=0):
    return tgt.at[idx].add(src)
def _segment_sum(src, seg, n):
    return jax.ops.segment_sum(src, seg, n)
class _Rng:
    def __init__(self, key):
        self._k = key
    def _next(self):
        self._k, sub = jax.random.split(self._k)
        return sub
    def normal(self, shape):
        return jax.random.normal(self._next(), shape, dtype=jnp.bfloat16)
    def randint(self, lo, hi, shape):
        return jax.random.randint(self._next(), shape, lo, hi, dtype=jnp.int32)
    def uniform(self, shape, lo=0.0, hi=1.0):
        return jax.random.uniform(self._next(), shape, jnp.bfloat16, lo, hi)
    def permutation(self, n):
        return jax.random.permutation(self._next(), n)


kernel_name = 'gated_mix__sliding_block_cached__dense_activation_gelu__decode'

def setup_inputs():
    _rng = _Rng(jax.random.key(int.from_bytes(__import__("os").urandom(4), "little")))
    _w = (lambda a: (lambda t: t.astype(jnp.bfloat16) if jnp.issubdtype(t.dtype, jnp.floating) else t)(jnp.asarray(a)))
    def _A_setup():
        B, Sq, D = 1, 1, 640
        Hq, Hkv, Sk, Dh = 32, 32, 32768, 192
        assert Hq % Hkv == 0, (Hq, Hkv)
        return {
            "x": _w((lambda *s: _rng.normal(s) * 0.05)(B, Sq, D)),
            "k_cache": _w((lambda *s: _rng.normal(s) * 0.05)(B, Hkv, Sk, Dh)),
            "v_cache": _w((lambda *s: _rng.normal(s) * 0.05)(B, Hkv, Sk, Dh)),
            "wq": _w((lambda *s: _rng.normal(s) * 0.05)(D, Hq * Dh) * (D ** -0.5)),
            "wo": _w((lambda *s: _rng.normal(s) * 0.05)(Hq * Dh, D) * ((Hq * Dh) ** -0.5)),
        }
    _A_in = _A_setup()

    def _B_setup():
        B, S, D, F = 1, 1, 640, 1536
        return {
            "x": _w((lambda *s: _rng.normal(s) * 0.05)(B, S, D)),
            "w1": _w((lambda *s: _rng.normal(s) * 0.05)(D, F) * (D ** -0.5)),
            "b1": _w((lambda *s: _rng.normal(s) * 0.05)(F) * 0.01),
            "w2": _w((lambda *s: _rng.normal(s) * 0.05)(F, D) * (F ** -0.5)),
            "b2": _w((lambda *s: _rng.normal(s) * 0.05)(D) * 0.01),
        }
    _B_in = _B_setup()

    return {
        "A_x": _A_in["x"],
        "A_k_cache": _A_in["k_cache"],
        "A_v_cache": _A_in["v_cache"],
        "A_wq": _A_in["wq"],
        "A_wo": _A_in["wo"],
        "B_x": _B_in["x"],
        "B_w1": _B_in["w1"],
        "B_b1": _B_in["b1"],
        "B_w2": _B_in["w2"],
        "B_b2": _B_in["b2"],
        "gate_w": _w((lambda *s: _rng.normal(s) * 0.05)(640)),
    }

def reference(A_x, A_k_cache, A_v_cache, A_wq, A_wo, B_x, B_w1, B_b1, B_w2, B_b2, gate_w):
    def _A_ref(x, k_cache, v_cache, wq, wo):
        B, Sq, D = x.shape
        Hq, Dh = 32, 192
        Hkv, Sk = k_cache.shape[1], k_cache.shape[2]
        W = min(4096, max(256, Sk // 4))
        rep = Hq // Hkv
        q = (lambda x, *d: x.transpose(*d))((x @ wq).reshape(B, Sq, Hq, Dh), 0, 2, 1, 3)
        k = jnp.repeat(k_cache[:, :, Sk - W:, :], rep, axis=1)
        v = jnp.repeat(v_cache[:, :, Sk - W:, :], rep, axis=1)
        scores = jnp.einsum("bhqd,bhkd->bhqk", q, k) * (Dh ** -0.5)
        p = _softmax(scores, axis=-1)
        o = jnp.einsum("bhqk,bhkd->bhqd", p, v)
        return (lambda x, *d: x.transpose(*d))(o, 0, 2, 1, 3).reshape(B, Sq, Hq * Dh) @ wo

    def _B_ref(x, w1, b1, w2, b2):
        h = jnp.einsum("bsd,df->bsf", x, w1) + b1
        h = _gelu(h)
        return jnp.einsum("bsf,fd->bsd", h, w2) + b2

    x = A_x
    g = _sigmoid((x * gate_w).sum(-1, keepdims=True))
    a = _A_ref(x, A_k_cache, A_v_cache, A_wq, A_wo)
    b = _B_ref(x, B_w1, B_b1, B_w2, B_b2)
    return g * a + (1 - g) * b
```

```python
import jax
import jax.numpy as jnp
from jax import lax
import jax.experimental.pallas as pl
import jax.experimental.pallas.tpu as pltpu

BF = jnp.bfloat16
F32 = jnp.float32
DEPTH = 3


@jax.jit
def pallas_gated_mix__sliding_block_cached__dense_activation_gelu__decode_kernel(
    A_x: jax.Array,
    A_k_cache: jax.Array,
    A_v_cache: jax.Array,
    A_wq: jax.Array,
    A_wo: jax.Array,
    B_x: jax.Array,
    B_w1: jax.Array,
    B_b1: jax.Array,
    B_w2: jax.Array,
    B_b2: jax.Array,
    gate_w: jax.Array,
):
    del B_x
    _, H, SK, DH = A_k_cache.shape
    D = A_x.shape[-1]
    F = B_w1.shape[1]
    W = min(4096, max(256, SK // 4))
    depth = DEPTH

    def kernel(x_hbm, k_hbm, v_hbm, wq_hbm, wo_hbm, w1_hbm, b1_hbm, w2_hbm, b2_hbm, g_hbm,
               o_ref,
               x_v, b1_v, b2_v, g_v, wq_v, w1_v, w2_v, kbuf, vbuf, wobuf, q_scr,
               ssem, ksem, vsem, wosem):
        cx = pltpu.make_async_copy(x_hbm, x_v, ssem.at[0])
        cb1 = pltpu.make_async_copy(b1_hbm, b1_v, ssem.at[1])
        cb2 = pltpu.make_async_copy(b2_hbm, b2_v, ssem.at[2])
        cg = pltpu.make_async_copy(g_hbm, g_v, ssem.at[3])
        cwq = pltpu.make_async_copy(wq_hbm, wq_v, ssem.at[4])
        cw1 = pltpu.make_async_copy(w1_hbm, w1_v, ssem.at[5])
        cw2 = pltpu.make_async_copy(w2_hbm, w2_v, ssem.at[6])

        def kcopy(h, slot):
            return pltpu.make_async_copy(k_hbm.at[0, h, :, pl.ds(SK - W, W)], kbuf.at[slot], ksem.at[slot])

        def vcopy(h, slot):
            return pltpu.make_async_copy(v_hbm.at[0, h, :, pl.ds(SK - W, W)], vbuf.at[slot], vsem.at[slot])

        def wocopy(h, slot):
            return pltpu.make_async_copy(wo_hbm.at[pl.ds(pl.multiple_of(h * DH, DH), DH), :], wobuf.at[slot], wosem.at[slot])

        cx.start()
        cwq.start()
        cb1.start()
        cb2.start()
        cg.start()
        cw1.start()
        for s in range(depth):
            kcopy(s, s).start()
            vcopy(s, s).start()
            wocopy(s, s).start()

        cx.wait()
        x = x_v[0]
        cwq.wait()
        q = jnp.dot(x, wq_v[...], preferred_element_type=F32)
        for h in range(H):
            q_scr[pl.ds(h, 1), :] = q[:, h * DH:(h + 1) * DH]

        scale = DH ** -0.5

        def head(h, acc):
            slot = h % depth
            qh = q_scr[pl.ds(h, 1), :].astype(BF)
            kcopy(h, slot).wait()
            s = jnp.dot(qh, kbuf[slot], preferred_element_type=F32) * scale
            m = jnp.max(s, axis=1, keepdims=True)
            p = jnp.exp(s - m)
            l = jnp.sum(p, axis=1, keepdims=True)
            vcopy(h, slot).wait()
            o = lax.dot_general(p.astype(BF), vbuf[slot], (((1,), (1,)), ((), ())), preferred_element_type=F32)
            o = (o / l).astype(BF)
            wocopy(h, slot).wait()
            acc = acc + jnp.dot(o, wobuf[slot], preferred_element_type=F32)

            @pl.when(h + depth < H)
            def _():
                kcopy(h + depth, slot).start()
                vcopy(h + depth, slot).start()
                wocopy(h + depth, slot).start()

            @pl.when(h + depth == H)
            def _():
                cw2.start()
            return acc

        a = lax.fori_loop(0, H, head, jnp.zeros((1, D), F32))

        cw1.wait()
        cb1.wait()
        hpre = jnp.dot(x, w1_v[...], preferred_element_type=F32) + b1_v[...].astype(F32).reshape(1, F)
        hact = jax.nn.gelu(hpre, approximate=True).astype(BF)
        cw2.wait()
        cb2.wait()
        cg.wait()
        b = jnp.dot(hact, w2_v[...], preferred_element_type=F32) + b2_v[...].astype(F32).reshape(1, D)
        gl = jnp.sum(x.astype(F32) * g_v[...].astype(F32).reshape(1, D), axis=1, keepdims=True)
        g = jax.nn.sigmoid(gl)
        o_ref[0] = (g * a + (1 - g) * b).astype(o_ref.dtype)

    kt = A_k_cache.transpose(0, 1, 3, 2)
    vt = A_v_cache.transpose(0, 1, 3, 2)
    hbm = pl.BlockSpec(memory_space=pltpu.HBM)
    return pl.pallas_call(
        kernel,
        out_shape=jax.ShapeDtypeStruct((1, 1, D), A_x.dtype),
        in_specs=[hbm] * 10,
        out_specs=pl.BlockSpec(memory_space=pltpu.VMEM),
        scratch_shapes=[
            pltpu.VMEM((1, 1, D), BF), pltpu.VMEM((F,), BF), pltpu.VMEM((D,), BF), pltpu.VMEM((D,), BF),
            pltpu.VMEM((D, H * DH), BF), pltpu.VMEM((D, F), BF), pltpu.VMEM((F, D), BF),
            pltpu.VMEM((depth, DH, W), BF), pltpu.VMEM((depth, DH, W), BF), pltpu.VMEM((depth, DH, D), BF),
            pltpu.VMEM((H, DH), F32),
            pltpu.SemaphoreType.DMA((7,)), pltpu.SemaphoreType.DMA((depth,)),
            pltpu.SemaphoreType.DMA((depth,)), pltpu.SemaphoreType.DMA((depth,)),
        ],
        compiler_params=pltpu.CompilerParams(vmem_limit_bytes=64 * 1024 * 1024),
    )(A_x, kt, vt, A_wq, A_wo, B_w1, B_b1, B_w2, B_b2, gate_w)
```

```python
import jax
import jax.numpy as jnp
from jax import lax
import jax.experimental.pallas as pl
import jax.experimental.pallas.tpu as pltpu

BF = jnp.bfloat16
F32 = jnp.float32

DEPTH = 2
W2_CHUNKS = (1024, 384, 128)
P_HI, P_LO = 0, 1


@jax.jit
def pallas_gated_mix__sliding_block_cached__dense_activation_gelu__decode_kernel(
    A_x: jax.Array,
    A_k_cache: jax.Array,
    A_v_cache: jax.Array,
    A_wq: jax.Array,
    A_wo: jax.Array,
    B_x: jax.Array,
    B_w1: jax.Array,
    B_b1: jax.Array,
    B_w2: jax.Array,
    B_b2: jax.Array,
    gate_w: jax.Array,
):
    del B_x
    _, H, SK, DH = A_k_cache.shape
    D = A_x.shape[-1]
    F = B_w1.shape[1]
    W = min(4096, max(256, SK // 4))
    depth = DEPTH
    w2_chunks = W2_CHUNKS
    assert sum(w2_chunks) == F and depth >= 2
    nchunk = len(w2_chunks)
    offs = [sum(w2_chunks[:i]) for i in range(nchunk)]

    def kernel(x_hbm, k_hbm, v_hbm, wq_hbm, wo_hbm, w1_hbm, b1_hbm, w2_hbm, b2_hbm, g_hbm,
               o_ref,
               x_v, b1_v, b2_v, g_v, wq_v, w1_v, w2_v, kbuf, vbuf, wobuf, q_scr,
               ssem, w2sem, ksem, vsem, wosem):
        cx = pltpu.make_async_copy(x_hbm, x_v, ssem.at[0])
        cb1 = pltpu.make_async_copy(b1_hbm, b1_v, ssem.at[1])
        cb2 = pltpu.make_async_copy(b2_hbm, b2_v, ssem.at[2])
        cg = pltpu.make_async_copy(g_hbm, g_v, ssem.at[3])
        cwq = pltpu.make_async_copy(wq_hbm, wq_v, ssem.at[4])
        cw1 = pltpu.make_async_copy(w1_hbm, w1_v, ssem.at[5])
        cw2 = [pltpu.make_async_copy(w2_hbm.at[pl.ds(o, n), :], w2_v.at[pl.ds(o, n), :], w2sem.at[i])
               for i, (o, n) in enumerate(zip(offs, w2_chunks))]

        def kcopy(h, slot):
            return pltpu.make_async_copy(
                k_hbm.at[0, h, :, pl.ds(SK - W, W)], kbuf.at[slot], ksem.at[slot])

        def vcopy(h, slot):
            return pltpu.make_async_copy(
                v_hbm.at[0, h, :, pl.ds(SK - W, W)], vbuf.at[slot], vsem.at[slot])

        def wocopy(h, slot):
            return pltpu.make_async_copy(
                wo_hbm.at[pl.ds(pl.multiple_of(h * DH, DH), DH), :], wobuf.at[slot], wosem.at[slot])

        def start_head(h, slot):
            kcopy(h, slot).start(priority=P_HI)
            vcopy(h, slot).start(priority=P_LO)
            wocopy(h, slot).start(priority=P_LO)

        cwq.start(priority=P_HI)
        cx.start(priority=P_HI)
        cw1.start(priority=P_HI)
        for s in range(depth):
            start_head(s, s)
        cb1.start(priority=P_HI)
        cb2.start(priority=P_HI)
        cg.start(priority=P_HI)

        cx.wait()
        x = x_v[0]
        cwq.wait()
        q = jnp.dot(x, wq_v[...], preferred_element_type=F32)
        for h in range(H):
            q_scr[pl.ds(h, 1), :] = q[:, h * DH:(h + 1) * DH]

        cw1.wait()
        cb1.wait()
        hpre = jnp.dot(x, w1_v[...], preferred_element_type=F32) + b1_v[...].astype(F32).reshape(1, F)
        hact = jax.nn.gelu(hpre, approximate=True).astype(BF)

        scale = DH ** -0.5

        def head(h, acc):
            slot = h % depth
            qh = q_scr[pl.ds(h, 1), :].astype(BF)
            kcopy(h, slot).wait()
            s = jnp.dot(qh, kbuf[slot], preferred_element_type=F32) * scale
            m = jnp.max(s, axis=1, keepdims=True)
            p = jnp.exp(s - m)
            l = jnp.sum(p, axis=1, keepdims=True)
            vcopy(h, slot).wait()
            o = lax.dot_general(p.astype(BF), vbuf[slot], (((1,), (1,)), ((), ())),
                                preferred_element_type=F32)
            o = (o / l).astype(BF)
            wocopy(h, slot).wait()
            acc = acc + jnp.dot(o, wobuf[slot], preferred_element_type=F32)

            @pl.when(h + depth < H)
            def _():
                start_head(h + depth, slot)

            for i in range(depth):
                @pl.when(h + depth == H + i)
                def _():
                    cw2[i].start(priority=P_LO)
            return acc

        a = lax.fori_loop(0, H, head, jnp.zeros((1, D), F32))

        cb2.wait()
        cg.wait()
        gl = jnp.sum(x.astype(F32) * g_v[...].astype(F32).reshape(1, D), axis=1, keepdims=True)
        g = jax.nn.sigmoid(gl)
        b = b2_v[...].astype(F32).reshape(1, D)
        started = depth
        for i, (o_, n) in enumerate(zip(offs, w2_chunks)):
            cw2[i].wait()
            if started < nchunk:
                cw2[started].start(priority=P_LO)
                started += 1
            b = b + jnp.dot(hact[:, o_:o_ + n], w2_v[pl.ds(o_, n), :], preferred_element_type=F32)
        o_ref[0] = (g * a + (1 - g) * b).astype(o_ref.dtype)

    kt = A_k_cache.transpose(0, 1, 3, 2)
    vt = A_v_cache.transpose(0, 1, 3, 2)
    hbm = pl.BlockSpec(memory_space=pltpu.HBM)
    return pl.pallas_call(
        kernel,
        out_shape=jax.ShapeDtypeStruct((1, 1, D), A_x.dtype),
        in_specs=[hbm] * 10,
        out_specs=pl.BlockSpec(memory_space=pltpu.VMEM),
        scratch_shapes=[
            pltpu.VMEM((1, 1, D), BF), pltpu.VMEM((F,), BF), pltpu.VMEM((D,), BF), pltpu.VMEM((D,), BF),
            pltpu.VMEM((D, H * DH), BF), pltpu.VMEM((D, F), BF), pltpu.VMEM((F, D), BF),
            pltpu.VMEM((depth, DH, W), BF), pltpu.VMEM((depth, DH, W), BF), pltpu.VMEM((depth, DH, D), BF),
            pltpu.VMEM((H, DH), F32),
            pltpu.SemaphoreType.DMA((6,)), pltpu.SemaphoreType.DMA((nchunk,)),
            pltpu.SemaphoreType.DMA((depth,)), pltpu.SemaphoreType.DMA((depth,)),
            pltpu.SemaphoreType.DMA((depth,)),
        ],
        compiler_params=pltpu.CompilerParams(
            vmem_limit_bytes=64 * 1024 * 1024,
            disable_bounds_checks=True,
            disable_semaphore_checks=True,
        ),
    )(A_x, kt, vt, A_wq, A_wo, B_w1, B_b1, B_w2, B_b2, gate_w)
```

```python
import jax
import jax.numpy as jnp
from jax import lax
import jax.experimental.pallas as pl
import jax.experimental.pallas.tpu as pltpu

BF = jnp.bfloat16
F32 = jnp.float32
LANES = 128

DEPTH = 3
W2_MXU_TAIL = 384
W2_VPU_CHUNKS = (96, 32)
P_HI, P_LO = 0, 1


@jax.jit
def pallas_gated_mix__sliding_block_cached__dense_activation_gelu__decode_kernel(
    A_x: jax.Array,
    A_k_cache: jax.Array,
    A_v_cache: jax.Array,
    A_wq: jax.Array,
    A_wo: jax.Array,
    B_x: jax.Array,
    B_w1: jax.Array,
    B_b1: jax.Array,
    B_w2: jax.Array,
    B_b2: jax.Array,
    gate_w: jax.Array,
):
    del B_x
    B, H, SK, DH = A_k_cache.shape
    D = A_x.shape[-1]
    F = B_w1.shape[1]
    W = min(4096, max(256, SK // 4))
    assert B == 1 and A_x.shape == (1, 1, D) and A_wq.shape == (D, H * DH)

    depth = DEPTH
    nvpu = sum(W2_VPU_CHUNKS)
    assert nvpu == LANES and depth >= 1
    w2_chunks = (F - nvpu - W2_MXU_TAIL, W2_MXU_TAIL) + W2_VPU_CHUNKS
    n_mxu = 2
    nchunk = len(w2_chunks)
    offs = [sum(w2_chunks[:i]) for i in range(nchunk)]
    n_inloop = min(depth, nchunk)

    def kernel(x_hbm, k_hbm, v_hbm, wq_hbm, wo_hbm, w1_hbm, b1_hbm, w2_hbm, b2_hbm, g_hbm,
               o_ref,
               x_v, b1_v, b2_v, g_v, wq_v, w1_v, w2_v, kbuf, vbuf, wobuf, q_scr, hcol,
               ssem, w2sem, ksem, vsem, wosem):
        cx = pltpu.make_async_copy(x_hbm, x_v, ssem.at[0])
        cb1 = pltpu.make_async_copy(b1_hbm, b1_v, ssem.at[1])
        cb2 = pltpu.make_async_copy(b2_hbm, b2_v, ssem.at[2])
        cg = pltpu.make_async_copy(g_hbm, g_v, ssem.at[3])
        cwq = pltpu.make_async_copy(wq_hbm, wq_v, ssem.at[4])
        cw1 = pltpu.make_async_copy(w1_hbm, w1_v, ssem.at[5])
        cw2 = [
            pltpu.make_async_copy(w2_hbm.at[pl.ds(o, n), :], w2_v.at[pl.ds(o, n), :], w2sem.at[i])
            for i, (o, n) in enumerate(zip(offs, w2_chunks))
        ]

        def kcopy(h, slot):
            return pltpu.make_async_copy(
                k_hbm.at[0, h, :, pl.ds(SK - W, W)], kbuf.at[slot], ksem.at[slot])

        def vcopy(h, slot):
            return pltpu.make_async_copy(
                v_hbm.at[0, h, :, pl.ds(SK - W, W)], vbuf.at[slot], vsem.at[slot])

        def wocopy(h, slot):
            rows = pl.ds(pl.multiple_of(h * DH, DH), DH)
            return pltpu.make_async_copy(wo_hbm.at[rows, :], wobuf.at[slot], wosem.at[slot])

        def start_head(h, slot):
            kcopy(h, slot).start(priority=P_HI)
            vcopy(h, slot).start(priority=P_LO)
            wocopy(h, slot).start(priority=P_LO)

        cwq.start(priority=P_HI)
        cx.start(priority=P_HI)
        cw1.start(priority=P_HI)
        for s in range(depth):
            start_head(s, s)
        cb1.start(priority=P_HI)
        cb2.start(priority=P_HI)
        cg.start(priority=P_HI)

        cx.wait()
        x = x_v[0]
        cwq.wait()
        q = jnp.dot(x, wq_v[...], preferred_element_type=F32)
        for h in range(H):
            q_scr[pl.ds(h, 1), :] = q[:, h * DH:(h + 1) * DH]

        cg.wait()
        gate = jax.nn.sigmoid(
            jnp.sum(x.astype(F32) * g_v[...].astype(F32).reshape(1, D), axis=1, keepdims=True))
        cw1.wait()
        cb1.wait()
        hpre = jnp.dot(x, w1_v[...], preferred_element_type=F32) + b1_v[...].astype(F32).reshape(1, F)
        hact = jax.nn.gelu(hpre, approximate=True).astype(BF)
        hlast = hact[:, F - nvpu:].astype(F32) * (1 - gate)
        hcol[...] = jnp.broadcast_to(hlast, (nvpu, nvpu)).T

        scale = DH ** -0.5

        def head(h, acc):
            slot = h % depth
            qh = q_scr[pl.ds(h, 1), :].astype(BF)
            kcopy(h, slot).wait()
            s = jnp.dot(qh, kbuf[slot], preferred_element_type=F32) * scale
            m = jnp.max(s, axis=1, keepdims=True)
            p = jnp.exp(s - m)
            l = jnp.sum(p, axis=1, keepdims=True)
            vcopy(h, slot).wait()
            o = lax.dot_general(p.astype(BF), vbuf[slot], (((1,), (1,)), ((), ())),
                                preferred_element_type=F32)
            o = (o / l).astype(BF)
            wocopy(h, slot).wait()
            acc = acc + jnp.dot(o, wobuf[slot], preferred_element_type=F32)

            @pl.when(h + depth < H)
            def _():
                start_head(h + depth, slot)

            for i in range(n_inloop):
                @pl.when(h + depth == H + i)
                def _():
                    cw2[i].start(priority=P_LO)
            return acc

        a = lax.fori_loop(0, H, head, jnp.zeros((1, D), F32))

        cb2.wait()
        b = b2_v[...].astype(F32).reshape(1, D)
        started = n_inloop
        for i, (o_, n) in enumerate(zip(offs, w2_chunks)):
            if i == n_mxu:
                mixed = gate * a + (1 - gate) * b
                row = lax.broadcasted_iota(jnp.int32, (8, D), 0)
                acc8 = jnp.where(row == 0, mixed, 0.0)
            cw2[i].wait()
            if started < nchunk:
                cw2[started].start(priority=P_LO)
                started += 1
            if i < n_mxu:
                b = b + jnp.dot(hact[:, o_:o_ + n], w2_v[pl.ds(o_, n), :],
                                preferred_element_type=F32)
            else:
                for r in range(0, n, 32):
                    hc = hcol[pl.ds(o_ - (F - nvpu) + r, 32), :]
                    prod = w2_v[pl.ds(o_ + r, 32), :].astype(F32) * jnp.tile(hc, (1, D // LANES))
                    for r8 in range(0, 32, 8):
                        acc8 = acc8 + prod[r8:r8 + 8]
        o_ref[0] = jnp.sum(acc8, axis=0, keepdims=True).astype(o_ref.dtype)

    kt = A_k_cache.transpose(0, 1, 3, 2)
    vt = A_v_cache.transpose(0, 1, 3, 2)
    hbm = pl.BlockSpec(memory_space=pltpu.HBM)
    return pl.pallas_call(
        kernel,
        out_shape=jax.ShapeDtypeStruct((1, 1, D), A_x.dtype),
        in_specs=[hbm] * 10,
        out_specs=pl.BlockSpec(memory_space=pltpu.VMEM),
        scratch_shapes=[
            pltpu.VMEM((1, 1, D), BF),
            pltpu.VMEM((F,), BF),
            pltpu.VMEM((D,), BF),
            pltpu.VMEM((D,), BF),
            pltpu.VMEM((D, H * DH), BF),
            pltpu.VMEM((D, F), BF),
            pltpu.VMEM((F, D), BF),
            pltpu.VMEM((depth, DH, W), BF),
            pltpu.VMEM((depth, DH, W), BF),
            pltpu.VMEM((depth, DH, D), BF),
            pltpu.VMEM((H, DH), F32),
            pltpu.VMEM((nvpu, nvpu), F32),
            pltpu.SemaphoreType.DMA((6,)),
            pltpu.SemaphoreType.DMA((nchunk,)),
            pltpu.SemaphoreType.DMA((depth,)),
            pltpu.SemaphoreType.DMA((depth,)),
            pltpu.SemaphoreType.DMA((depth,)),
        ],
        compiler_params=pltpu.CompilerParams(
            vmem_limit_bytes=64 * 1024 * 1024,
            disable_bounds_checks=True,
            disable_semaphore_checks=True,
        ),
    )(A_x, kt, vt, A_wq, A_wo, B_w1, B_b1, B_w2, B_b2, gate_w)
```
